```python
import os as _os
_os.environ.setdefault('JAX_PLATFORMS', 'cpu')
import jax
import jax.numpy as jnp

def _softmax(x, axis=-1):
    return jax.nn.softmax(x, axis=axis)

def _gelu(x):
    return jax.nn.gelu(x, approximate=True)

def _silu(x):
    return jax.nn.silu(x)

def _sigmoid(x):
    return jax.nn.sigmoid(x)

def _layernorm(x, axis=-1, eps=1e-05):
    m = jnp.mean(x, axis=axis, keepdims=True)
    v = jnp.var(x, axis=axis, keepdims=True)
    return (x - m) / jnp.sqrt(v + eps)

def _scatter_add(tgt, idx, src, axis=0):
    return tgt.at[idx].add(src)

def _segment_sum(src, seg, n):
    return jax.ops.segment_sum(src, seg, n)

class _Rng:

    def __init__(self, key):
        self._k = key

    def _next(self):
        self._k, sub = jax.random.split(self._k)
        return sub

    def normal(self, shape):
        return jax.random.normal(self._next(), shape, dtype=jnp.bfloat16)

    def randint(self, lo, hi, shape):
        return jax.random.randint(self._next(), shape, lo, hi, dtype=jnp.int32)

    def uniform(self, shape, lo=0.0, hi=1.0):
        return jax.random.uniform(self._next(), shape, jnp.bfloat16, lo, hi)

    def permutation(self, n):
        return jax.random.permutation(self._next(), n)
kernel_name = 'parallel_sum__memory_aug_recurrent_mem_tr__dense_activation_gelu__prompt'

def setup_inputs():
    _rng = _Rng(jax.random.key(int.from_bytes(__import__("os").urandom(4), "little")))
    _w = lambda a: (lambda t: t.astype(jnp.bfloat16) if jnp.issubdtype(t.dtype, jnp.floating) else t)(jnp.asarray(a))

    def _A_setup():
        B, S, Dm = (1, 2048, 1024)
        H, Dh = (32, 128)
        M, seg = (8, 32)
        seg = min(seg, S)
        S = S // seg * seg
        return {'x': _w((lambda *s: _rng.normal(s) * 0.05)(B, S, Dm)), 'mem0': _w((lambda *s: _rng.normal(s) * 0.2)(B, M, Dm)), 'Wq': _w((lambda *s: _rng.normal(s) * 0.8)(Dm, H, Dh) * Dm ** (-0.5)), 'Wk': _w((lambda *s: _rng.normal(s) * 0.8)(Dm, H, Dh) * Dm ** (-0.5)), 'Wv': _w((lambda *s: _rng.normal(s) * 0.2)(Dm, H, Dh) * Dm ** (-0.5)), 'Wo': _w((lambda *s: _rng.normal(s) * 0.2)(H, Dh, Dm) * (H * Dh) ** (-0.5)), 'seg_len': seg}
    _A_in = _A_setup()

    def _B_setup():
        B, S, D, F = (1, 2048, 1024, 3584)
        return {'x': _w((lambda *s: _rng.normal(s) * 0.05)(B, S, D)), 'w1': _w((lambda *s: _rng.normal(s) * 0.1)(D, F) * D ** (-0.5)), 'b1': _w((lambda *s: _rng.normal(s) * 0.1)(F) * 0.01), 'w2': _w((lambda *s: _rng.normal(s) * 0.1)(F, D) * F ** (-0.5)), 'b2': _w((lambda *s: _rng.normal(s) * 0.05)(D) * 0.01)}
    _B_in = _B_setup()
    return {'A_x': _A_in['x'], 'A_mem0': _A_in['mem0'], 'A_Wq': _A_in['Wq'], 'A_Wk': _A_in['Wk'], 'A_Wv': _A_in['Wv'], 'A_Wo': _A_in['Wo'], 'A_seg_len': _A_in['seg_len'], 'B_x': _B_in['x'], 'B_w1': _B_in['w1'], 'B_b1': _B_in['b1'], 'B_w2': _B_in['w2'], 'B_b2': _B_in['b2']}

def reference(A_x, A_mem0, A_Wq, A_Wk, A_Wv, A_Wo, A_seg_len, B_x, B_w1, B_b1, B_w2, B_b2):

    def _A_ref(x, mem0, Wq, Wk, Wv, Wo, seg_len):
        B, S, Dm = x.shape
        H, Dh = (Wq.shape[1], Wq.shape[2])
        M = mem0.shape[1]
        scale = Dh ** (-0.5)
        n_seg = S // seg_len
        L = M + seg_len
        idx = jnp.arange(L)
        mask = (idx[:, None] < M) | (idx[:, None] >= idx[None, :])
        mem = mem0
        outs = []
        for s in range(n_seg):
            xs = x[:, s * seg_len:(s + 1) * seg_len, :].copy()
            h = jnp.concatenate([mem, xs], axis=1)
            q = jnp.einsum('btd,dhe->bhte', h, Wq)
            k = jnp.einsum('btd,dhe->bhte', h, Wk)
            v = jnp.einsum('btd,dhe->bhte', h, Wv)
            scores = jnp.einsum('bhqe,bhke->bhqk', q, k) * scale
            scores = jnp.where(mask[None, None], scores, -1000000000.0)
            p = _softmax(scores, axis=-1)
            o = jnp.einsum('bhqk,bhke->bhqe', p, v)
            o = jnp.einsum('bhte,hed->btd', o, Wo)
            mem = o[:, :M, :].copy()
            outs.append(o[:, M:, :])
        return jnp.concatenate(outs, axis=1)

    def _B_ref(x, w1, b1, w2, b2):
        h = jnp.einsum('bsd,df->bsf', x, w1) + b1
        h = _gelu(h)
        return jnp.einsum('bsf,fd->bsd', h, w2) + b2
    x = A_x
    xn = _layernorm(x, axis=-1)
    return x + _A_ref(xn, A_mem0, A_Wq, A_Wk, A_Wv, A_Wo, A_seg_len) + _B_ref(xn, B_w1, B_b1, B_w2, B_b2)
```

```python
import functools
import jax
import jax.numpy as jnp
from jax import lax
import jax.experimental.pallas as pl
import jax.experimental.pallas.tpu as pltpu

S, D, H, DH, M, SEG, F = 2048, 1024, 32, 128, 8, 32, 3584
NSEG = S // SEG
L0 = 544
R = 576
G = 24
RD = R
LOG2E = 1.4426950408889634
QS = DH ** -0.5 * LOG2E
NEG = -1e9
bf16, f32, i32 = jnp.bfloat16, jnp.float32, jnp.int32
FC = 896
BM = 512
NC = F // FC
NR = S // BM
RAWD = 80
NRAW = 13


def gelu_tanh(x):
    c = 0.7978845608028654
    return 0.5 * x * (1.0 + jnp.tanh(c * (x + 0.044715 * (x * x * x))))


def dot(a, b):
    return jnp.dot(a, b, preferred_element_type=f32)


def make_kernel(cfg):
    def kernel(x_hbm, mem0_hbm, wq_hbm, wk_hbm, wv_hbm, wo_hbm, w1_hbm, b1_hbm, w2_hbm, b2_hbm,
               out_hbm,
               wqp, wkp, wvp, wop, w1p, w2p, xs, xn_ref, acc_ref, stg, qr, kr, vr, orr, out_s,
               mem0_s, b1_s, b2_s, b1c, b2r,
               sem_x, sem_w1, sem_w2, sem_raw, sem_misc, sem_out):
        def cp_x(r):
            return pltpu.make_async_copy(x_hbm.at[pl.ds(r * BM, BM), :], xs.at[pl.ds(r * BM, BM), :], sem_x.at[r])

        def cp_w1(c):
            return pltpu.make_async_copy(w1_hbm.at[:, pl.ds(c * FC, FC)], w1p.bitcast(bf16).at[:, pl.ds(c * FC, FC)], sem_w1.at[c])

        def cp_w2(c):
            return pltpu.make_async_copy(w2_hbm.at[pl.ds(c * FC, FC), :], w2p.bitcast(bf16).at[pl.ds(c * FC, FC), :], sem_w2.at[c])

        def raw_d0(k):
            return pl.multiple_of(jnp.minimum(k * RAWD, D - RAWD), 16)

        def cp_raw(k, m):
            src = (wq_hbm, wk_hbm, wv_hbm)[m]
            slot = lax.rem(k, 2) if not isinstance(k, int) else k % 2
            return pltpu.make_async_copy(src.at[pl.ds(pl.multiple_of(raw_d0(k) * H, 512), RAWD * H), :],
                                         stg.at[slot, m].bitcast(bf16), sem_raw.at[slot, m])

        cp_wo = pltpu.make_async_copy(wo_hbm, wop.bitcast(bf16), sem_misc.at[0])
        cp_mem = pltpu.make_async_copy(mem0_hbm, mem0_s, sem_misc.at[1])
        cp_b1 = pltpu.make_async_copy(b1_hbm, b1_s, sem_misc.at[2])
        cp_b2 = pltpu.make_async_copy(b2_hbm, b2_s, sem_misc.at[3])

        cp_x(0).start()
        cp_b2.start()
        cp_b1.start()
        cp_w1(0).start()
        cp_mem.start()

        def ln(row0, n, dst0):
            x = xs[pl.ds(row0, n), :].astype(f32)
            mu = jnp.mean(x, axis=-1, keepdims=True)
            xc = x - mu
            var = jnp.mean(xc * xc, axis=-1, keepdims=True)
            xn_ref[pl.ds(dst0, n), :] = (xc * lax.rsqrt(var + 1e-5)).astype(bf16)
            acc_ref[pl.ds(dst0, n), :] = x + b2r[...]

        cp_b2.wait()
        b2r[...] = b2_s[...].astype(f32).reshape(1, D)
        cp_x(0).wait()
        cp_w2(0).start()
        lax.fori_loop(0, 4, lambda j, c: (ln(pl.multiple_of(j * 128, 128), 128, pl.multiple_of(j * 128, 128)), c)[1], 0)
        cp_x(1).start()
        cp_b1.wait()
        b1v = b1_s[...].astype(f32).reshape(1, F)
        for c in range(NC):
            b1c[c] = b1v[:, c * FC:(c + 1) * FC]

        def relayout_part(k, parts):
            slot = lax.rem(k, 2)
            d0 = raw_d0(k)
            for (m, g, hp) in parts:
                dst = (wqp, wkp, wvp)[m]
                rows = pl.ds(pl.multiple_of(d0 // 2 + g * 8, 8), 8)
                z = stg[slot, m, pl.ds(g * 256 + hp, 16, stride=16), :]
                dst[2 * hp, rows, :] = pltpu.bitcast(z.astype(jnp.int16), i32)
                dst[2 * hp + 1, rows, :] = pltpu.bitcast((z >> 16).astype(jnp.int16), i32)

        all_parts = [(m, g, hp) for m in range(3) for g in range(RAWD // 16) for hp in range(H // 2)]

        def ffn(i, carry):
            r = i // NC
            c = i % NC

            @pl.when(r == 0)
            def _():
                cp_w1(c).wait()
                cp_w2(c).wait()

            @pl.when((r == 0) & (c < NC - 1))
            def _():
                cp_w1(c + 1).start()
                cp_w2(c + 1).start()

            @pl.when((c == 0) & (r < NR - 1))
            def _():
                cp_x(r + 1).wait()

            @pl.when((c == 1) & (r < NR - 2))
            def _():
                cp_x(r + 2).start()

            k = i - 3

            @pl.when(k >= 0)
            def _():
                for m in range(3):
                    cp_raw(k, m).wait()

            @pl.when((k + 1 >= 0) & (k + 1 < NRAW))
            def _():
                for m in range(3):
                    cp_raw(k + 1, m).start()

            @pl.when(i == 4)
            def _():
                cp_wo.start()

            kk = jnp.maximum(k, 0)
            rows = pl.ds(pl.multiple_of(r * BM, BM), BM)
            nr = jnp.minimum(r + 1, NR - 1)
            src = pl.multiple_of(nr * BM + c * 128, 128)
            dst = pl.multiple_of(jnp.where(r + 1 < NR, src, S), 128)
            NT = FC // 128
            nslots = NT + D // 128
            LNR = cfg.get('lnr', 16)
            extra = [[] for _ in range(nslots)]
            mode = cfg.get('il', 'spread')
            for idx, p in enumerate(all_parts):
                if mode == 'spread':
                    extra[idx * nslots // len(all_parts)].append(p)
            do_ln = cfg.get('ln_in', True)

            def side(slot):
                if cfg.get('relayout_in', True):
                    relayout_part(kk, extra[slot])
                if do_ln and slot < 128 // LNR:
                    ln(src + slot * LNR, LNR, dst + slot * LNR)

            xb = xn_ref[rows, :]
            hs = []
            for j in range(NT):
                cols = pl.ds(pl.multiple_of(c * FC + j * 128, 128), 128)
                hj = dot(xb, pltpu.bitcast(w1p[:, cols], bf16)) + b1c[c, :, j * 128:(j + 1) * 128]
                hs.append(gelu_tanh(hj).astype(bf16))
                side(j)
            h = jnp.concatenate(hs, axis=1)
            for n in range(D // 128):
                w2v = pltpu.bitcast(w2p[pl.ds(pl.multiple_of(c * (FC // 2), 8), FC // 2), n * 128:(n + 1) * 128], bf16)
                acc_ref[rows, n * 128:(n + 1) * 128] += dot(h, w2v)
                side(NT + n)
            return carry

        if cfg.get('ffn', True):
            lax.fori_loop(0, NR * NC, ffn, 0)

        if cfg.get('pre', True):
            PH = cfg.get('pre_heads', 1)

            def pre(hh, c):
                lhs = xn_ref[0:L0, :]
                for j in range(PH):
                    h = hh * PH + j
                    q = dot(lhs, pltpu.bitcast(wqp[h], bf16)) * QS
                    qr[h, 0:L0, :] = q.astype(bf16)
                    kr[h, 0:L0, :] = dot(lhs, pltpu.bitcast(wkp[h], bf16)).astype(bf16)
                    vr[h, 0:L0, :] = dot(lhs, pltpu.bitcast(wvp[h], bf16)).astype(bf16)
                    orr[h, 0:32, :] = jnp.zeros((32, DH), bf16)
                return c
            lax.fori_loop(0, H // PH, pre, 0)

        cp_wo.wait()
        cp_mem.wait()

        rowi = lax.broadcasted_iota(i32, (40, 48), 0)
        coli = lax.broadcasted_iota(i32, (40, 48), 1)
        mask = (coli < 40) & ((rowi >= SEG) | (coli >= SEG) | (coli <= rowi))
        z8 = jnp.zeros((8, DH), f32)

        def cp_out(row0, n):
            return pltpu.make_async_copy(out_s.at[pl.ds(row0, n), :], out_hbm.at[pl.ds(row0, n), :], sem_out)

        def step(s, mem):
            @pl.when(s >= 2)
            def _():
                cp_out(pl.multiple_of(G * (s - 2), 8), G).start()

            xrow = [L0 + G * s + 8 * i for i in range(3)]
            xsrc = [pl.multiple_of(jnp.minimum(r, S - 8), 8) for r in xrow]
            xslot = [pl.multiple_of(jnp.where(r < S, lax.rem(r, R), RD), 8) for r in xrow]
            orow = [jnp.maximum(G * (s - 1) + 8 * i, 0) for i in range(3)]
            oslot = [pl.multiple_of(lax.rem(r, R), 8) for r in orow]
            sslot = pl.multiple_of(lax.rem(SEG * s, R), SEG)
            seg = pl.ds(sslot, SEG)
            lhs = jnp.concatenate([mem] + [xn_ref[pl.ds(r, 8), :].astype(f32) for r in xsrc], axis=0).astype(bf16)
            st = {}

            def pad16(a):
                return jnp.concatenate([a, z8], axis=0).astype(bf16)

            def qkv(h):
                q = dot(lhs, pltpu.bitcast(wqp[h], bf16)) * QS
                k = dot(lhs, pltpu.bitcast(wkp[h], bf16))
                v = dot(lhs, pltpu.bitcast(wvp[h], bf16))
                for i in range(3):
                    sl = pl.ds(xslot[i], 8)
                    qr[h, sl, :] = q[8 * (i + 1):8 * (i + 2)].astype(bf16)
                    kr[h, sl, :] = k[8 * (i + 1):8 * (i + 2)].astype(bf16)
                    vr[h, sl, :] = v[8 * (i + 1):8 * (i + 2)].astype(bf16)
                st['qm', h], st['km', h], st['vm', h] = pad16(q[0:8]), pad16(k[0:8]), pad16(v[0:8])

            def ld_qk(h):
                st['qx', h] = qr[h, seg, :]
                st['kx', h] = kr[h, seg, :]

            def ld_v(h):
                st['vx', h] = vr[h, seg, :]

            def ld_o(h):
                st['og', h] = [orr[h, pl.ds(oslot[i], 8), :].astype(f32) for i in range(3)]

            def qk(h):
                q_all = jnp.concatenate([st.pop(('qx', h)), st.pop(('qm', h))], axis=0)
                k_all = jnp.concatenate([st.pop(('kx', h)), st.pop(('km', h))], axis=0)
                sc = lax.dot_general(q_all, k_all, (((1,), (1,)), ((), ())), preferred_element_type=f32)[0:40]
                sc = jnp.where(mask, sc, NEG)
                mx = jnp.max(sc, axis=1, keepdims=True)
                p = jnp.exp2(sc - mx)
                l = jnp.sum(p, axis=1, keepdims=True)
                st['p', h] = jnp.concatenate([p, jnp.zeros((8, 48), f32)], axis=0).astype(bf16)
                r = pl.reciprocal(l, approx=True)
                st['il', h] = r * (2.0 - l * r)

            def pv(h):
                v_all = jnp.concatenate([st.pop(('vx', h)), st.pop(('vm', h))], axis=0)
                o = dot(st.pop(('p', h)), v_all)[0:40] * st.pop(('il', h))
                orr[h, seg, :] = o[0:32].astype(bf16)
                st['lo', h] = jnp.concatenate([o[32:40]] + st.pop(('og', h)), axis=0).astype(bf16)

            def wo(h):
                t = dot(st.pop(('lo', h)), pltpu.bitcast(wop[h], bf16))
                st['acc'] = t if 'acc' not in st else st['acc'] + t

            a, b, c = cfg.get('skew', (1, 2, 3))
            for t in range(H + c):
                if 0 <= t - a < H: ld_qk(t - a)
                if 0 <= t - b < H: ld_v(t - b); ld_o(t - b)
                if t < H: qkv(t)
                if 0 <= t - a < H: qk(t - a)
                if 0 <= t - b < H: pv(t - b)
                if 0 <= t - c < H: wo(t - c)
            acc = st['acc']
            for i in range(3):
                rr = pl.ds(pl.multiple_of(jnp.where(s > 0, orow[i], S), 8), 8)
                out_s[rr, :] = (acc_ref[rr, :] + acc[8 * (i + 1):8 * (i + 2)]).astype(bf16)
            return acc[0:8].astype(bf16).astype(f32)

        mem = mem0_s[...].astype(f32)
        if cfg.get('loop', True):
            lax.fori_loop(0, NSEG, step, mem)

        P0 = 1504
        PN = (S - P0) // 2

        def post(j, c):
            row0 = P0 + j * PN
            lo = jnp.concatenate(
                [jnp.concatenate([orr[h, pl.ds(pl.multiple_of(lax.rem(row0 + 16 * g, R), 16), 16), :] for g in range(PN // 16)], axis=0)
                 for h in range(H)], axis=1)
            t = dot(lo, pltpu.bitcast(wop[...].reshape(H * DH // 2, D), bf16))
            rr = pl.ds(pl.multiple_of(row0, 16), PN)
            out_s[rr, :] = (acc_ref[rr, :] + t).astype(bf16)
            return c
        if cfg.get('post', True):
            lax.fori_loop(0, 2, post, 0)
        cp_out(G * (NSEG - 2), S - G * (NSEG - 2)).start()
        pltpu.make_async_copy(out_s.at[pl.ds(0, S), :], out_hbm, sem_out).wait()

    return kernel


def build(cfg=None):
    cfg = cfg or {}

    @jax.jit
    def fn(A_x, A_mem0, A_Wq, A_Wk, A_Wv, A_Wo, A_seg_len, B_x, B_w1, B_b1, B_w2, B_b2):
        hbm = pl.BlockSpec(memory_space=pltpu.HBM)
        out = pl.pallas_call(
            make_kernel(cfg),
            out_shape=jax.ShapeDtypeStruct((S, D), bf16),
            in_specs=[hbm] * 10,
            out_specs=hbm,
            scratch_shapes=[
                pltpu.VMEM((H, D // 2, DH), i32), pltpu.VMEM((H, D // 2, DH), i32), pltpu.VMEM((H, D // 2, DH), i32),
                pltpu.VMEM((H, DH // 2, D), i32),
                pltpu.VMEM((D // 2, F), i32), pltpu.VMEM((F // 2, D), i32),
                pltpu.VMEM((S, D), bf16), pltpu.VMEM((S + 128, D), bf16), pltpu.VMEM((S + 128, D), f32),
                pltpu.VMEM((2, 3, RAWD * H // 2, DH), i32),
                pltpu.VMEM((H, R + 16, DH), bf16), pltpu.VMEM((H, R + 16, DH), bf16), pltpu.VMEM((H, R + 16, DH), bf16),
                pltpu.VMEM((H, R + 16, DH), bf16),
                pltpu.VMEM((S + 16, D), bf16),
                pltpu.VMEM((M, D), bf16), pltpu.VMEM((F,), bf16), pltpu.VMEM((D,), bf16),
                pltpu.VMEM((NC, 1, FC), f32), pltpu.VMEM((1, D), f32),
                pltpu.SemaphoreType.DMA((NR,)), pltpu.SemaphoreType.DMA((NC,)), pltpu.SemaphoreType.DMA((NC,)),
                pltpu.SemaphoreType.DMA((2, 3)), pltpu.SemaphoreType.DMA((4,)), pltpu.SemaphoreType.DMA(()),
            ],
            compiler_params=pltpu.CompilerParams(vmem_limit_bytes=110 * 1024 * 1024),
            name="fused",
        )(A_x.reshape(S, D), A_mem0.reshape(M, D), A_Wq.reshape(D * H, DH), A_Wk.reshape(D * H, DH),
          A_Wv.reshape(D * H, DH), A_Wo, B_w1, B_b1, B_w2, B_b2)
        return out.reshape(1, S, D)
    return fn


_fn = build()


@jax.jit
def pallas_parallel_sum__memory_aug_recurrent_mem_tr__dense_activation_gelu__prompt_kernel(A_x, A_mem0, A_Wq, A_Wk, A_Wv, A_Wo, A_seg_len, B_x, B_w1, B_b1, B_w2, B_b2):
    return _fn(A_x, A_mem0, A_Wq, A_Wk, A_Wv, A_Wo, A_seg_len, B_x, B_w1, B_b1, B_w2, B_b2)
```

```python
import jax
import jax.numpy as jnp
from jax import lax
import jax.experimental.pallas as pl
import jax.experimental.pallas.tpu as pltpu

S, D, H, DH, M, SEG, F = 2048, 1024, 32, 128, 8, 32, 3584
NSEG = S // SEG
G = 24
L0 = 512
R = 576
PB = 128

BM, FC = 512, 896
NR, NC = S // BM, F // FC
NT = FC // 128
LNT = 256
XS = 4
W1S = (0, 1, 3, NT)
RAWD, NRAW = 80, 13
RAW0 = 3

LOG2E = 1.4426950408889634
QSCALE = DH ** -0.5 * LOG2E
MASKED = -1e9 * LOG2E

bf16, f32, i32 = jnp.bfloat16, jnp.float32, jnp.int32


def _gelu(x):
    c = 0.7978845608028654
    return 0.5 * x * (1.0 + jnp.tanh(c * (x + 0.044715 * (x * x * x))))


def _dot(a, b):
    return jnp.dot(a, b, preferred_element_type=f32)


def _step_schedule():
    a, b, c = 1, 3, 6
    ops, nq, nw = [], 0, 0
    for t in range(H // 2):
        for ch in "ADBADC":
            if ch == "A":
                ops.append(("qkv", nq))
                nq += 1
            elif ch == "B" and t >= a:
                ops.append(("qk", t - a))
            elif ch == "C" and t >= b:
                ops.append(("pv", t - b))
            elif ch == "D" and t >= c:
                ops.append(("wo", nw))
                nw += 1
    qk = list(range(H // 2 - a, H // 2))
    pv = list(range(H // 2 - b, H // 2))
    nf = 0
    for ch in "ppwwwqwwwwpwwwwwffffffff":
        if ch == "q":
            ops.append(("qk", qk.pop(0)))
        elif ch == "p":
            ops.append(("pv", pv.pop(0)))
        elif ch == "w":
            ops.append(("wo", nw))
            nw += 1
        else:
            ops.append(("fill", nf))
            nf += 1
    assert not qk and not pv and nq == H and nw == H and nf == H // 4
    return ops


def _kernel(x_hbm, mem0_hbm, wq_hbm, wk_hbm, wv_hbm, wo_hbm, w1_hbm, b1_hbm, w2_hbm, b2_hbm,
            out_hbm,
            wqp, wkp, wvp, wop, w1p, w2p, stg,
            xs, xn_ref, acc_ref, hs_ref, facc_ref, out_s,
            qr, kr, vr, orr,
            mem0_s, b1_s, b2_s, b1c, b2r,
            sem_x, sem_x0, sem_w1, sem_w1f, sem_w2, sem_raw, sem_misc, sem_out):

    def cp_x(r):
        rows = pl.ds(r * BM, BM)
        return pltpu.make_async_copy(x_hbm.at[rows, :], xs.at[rows, :], sem_x.at[r])

    def cp_x0(p):
        rows = pl.ds(p * (BM // XS), BM // XS)
        return pltpu.make_async_copy(x_hbm.at[rows, :], xs.at[rows, :], sem_x0.at[p])

    def cp_w1(c):
        cols = pl.ds(c * FC, FC)
        return pltpu.make_async_copy(w1_hbm.at[:, cols], w1p.bitcast(bf16).at[:, cols], sem_w1.at[c])

    def cp_w1f(p):
        cols = pl.ds(W1S[p] * 128, (W1S[p + 1] - W1S[p]) * 128)
        return pltpu.make_async_copy(w1_hbm.at[:, cols], w1p.bitcast(bf16).at[:, cols], sem_w1f.at[p])

    def cp_w2(c):
        rows = pl.ds(c * FC, FC)
        return pltpu.make_async_copy(w2_hbm.at[rows, :], w2p.bitcast(bf16).at[rows, :], sem_w2.at[c])

    def raw_d0(k):
        if isinstance(k, int):
            return min(k * RAWD, D - RAWD)
        return pl.multiple_of(jnp.minimum(k * RAWD, D - RAWD), 16)

    def cp_raw(k, m):
        row0 = raw_d0(k) * H
        if not isinstance(k, int):
            row0 = pl.multiple_of(row0, 16 * H)
        return pltpu.make_async_copy((wq_hbm, wk_hbm, wv_hbm)[m].at[pl.ds(row0, RAWD * H), :],
                                     stg.at[k, m].bitcast(bf16), sem_raw.at[k])

    def cp_out(row0, n):
        rows = pl.ds(row0, n)
        return pltpu.make_async_copy(out_s.at[rows, :], out_hbm.at[rows, :], sem_out)

    cp_wo = pltpu.make_async_copy(wo_hbm, wop.bitcast(bf16), sem_misc.at[0])
    cp_mem = pltpu.make_async_copy(mem0_hbm, mem0_s, sem_misc.at[1])
    cp_b1 = pltpu.make_async_copy(b1_hbm, b1_s, sem_misc.at[2])
    cp_b2 = pltpu.make_async_copy(b2_hbm, b2_s, sem_misc.at[3])

    cp_b2.start()
    cp_b1.start()
    cp_mem.start()
    for p in range(XS):
        cp_x0(p).start()
    for p in range(len(W1S) - 1):
        cp_w1f(p).start()
    cp_w2(0).start()
    cp_w1(1).start()
    cp_w2(1).start()
    cp_x(1).start()
    for c in range(2, NC):
        cp_w1(c).start()
        cp_w2(c).start()
    for r in range(2, NR):
        cp_x(r).start()

    def layernorm(row0, n, dst0):
        x = xs[pl.ds(row0, n), :].astype(f32)
        mu = jnp.mean(x, axis=-1, keepdims=True)
        xc = x - mu
        var = jnp.mean(xc * xc, axis=-1, keepdims=True)
        xn_ref[pl.ds(dst0, n), :] = (xc * lax.rsqrt(var + 1e-5)).astype(bf16)

    def deinterleave(krel, parts):
        d0 = raw_d0(jnp.maximum(krel, 0))
        k = jnp.where(krel < 0, NRAW, krel)
        for (m, g, hp) in parts:
            dst = (wqp, wkp, wvp)[m]
            rows = pl.ds(pl.multiple_of(d0 // 2 + g * 8, 8), 8)
            z = stg[k, m, pl.ds(g * 256 + hp, 16, stride=16), :]
            dst[2 * hp, rows, :] = pltpu.bitcast(z.astype(jnp.int16), i32)
            dst[2 * hp + 1, rows, :] = pltpu.bitcast((z >> 16).astype(jnp.int16), i32)

    nslots = NT + D // 128
    all_parts = [(m, g, hp) for m in range(3) for g in range(RAWD // 16) for hp in range(H // 2)]
    slot_parts = [[] for _ in range(nslots)]
    for idx, part in enumerate(all_parts):
        slot_parts[2 + idx * (nslots - 4) // len(all_parts)].append(part)

    for m in range(3):
        stg[NRAW, m] = jnp.zeros((RAWD * H // 2, DH), i32)
    cp_b2.wait()
    b2r[...] = b2_s[...].astype(f32).reshape(1, D)
    cp_b1.wait()
    b1v = b1_s[...].astype(f32).reshape(1, F)
    for c in range(NC):
        b1c[c] = b1v[:, c * FC:(c + 1) * FC]
    for p in range(XS):
        cp_x0(p).wait()
        for j in range(BM // XS // 128):
            layernorm(p * (BM // XS) + j * 128, 128, p * (BM // XS) + j * 128)
    for k in range(NRAW):
        for m in range(3):
            cp_raw(k, m).start()

    def ffn(i, carry, first=False):
        r, c = i // NC, i % NC
        k = i - RAW0
        if not first:
            @pl.when(r == 0)
            def _():
                cp_w1(c).wait()
                cp_w2(c).wait()

            @pl.when((c == NC - BM // LNT) & (r < NR - 1))
            def _():
                cp_x(r + 1).wait()

            @pl.when(k >= 0)
            def _():
                for m in range(3):
                    cp_raw(k, m).wait()

            @pl.when(i == 2)
            def _():
                cp_wo.start()

            lnv = (r + 1 < NR) & (c >= NC - BM // LNT)
            src = pl.multiple_of(
                jnp.where(lnv, (r + 1) * BM + (c - (NC - BM // LNT)) * LNT, r * BM), 16)
            dst = pl.multiple_of(jnp.where(lnv, src, S), 16)

        def side(slot):
            if first:
                return
            deinterleave(k, slot_parts[slot])
            if slot == 3:
                layernorm(src, LNT, dst)

        rows = pl.ds(pl.multiple_of(r * BM, BM), BM)
        xb = xn_ref[rows, :]
        for j in range(NT):
            if first and j in W1S:
                cp_w1f(W1S.index(j)).wait()
            cols = pl.ds(pl.multiple_of(c * FC + j * 128, 128), 128)
            hj = _dot(xb, pltpu.bitcast(w1p[:, cols], bf16)) + b1c[c, :, j * 128:(j + 1) * 128]
            hs_ref[:, j * 128:(j + 1) * 128] = pltpu.bitcast(_gelu(hj).astype(bf16), i32)
            side(j)
        if first:
            cp_w2(0).wait()
        h = pltpu.bitcast(hs_ref[...], bf16)
        for n in range(D // 128):
            ncols = slice(n * 128, (n + 1) * 128)
            w2v = pltpu.bitcast(w2p[pl.ds(pl.multiple_of(c * (FC // 2), 8), FC // 2), ncols], bf16)
            if first:
                base = b2r[:, ncols]
            else:
                base = jnp.where(c == 0, jnp.broadcast_to(b2r[:, ncols], (BM, 128)), acc_ref[rows, ncols])
            acc_ref[rows, ncols] = base + _dot(h, w2v)
            side(NT + n)
        return carry

    ffn(0, 0, first=True)
    lax.fori_loop(1, NR * NC, ffn, 0)

    def pre(j, carry):
        rows = pl.ds(pl.multiple_of(j * PB, PB), PB)
        lhs = xn_ref[rows, :]
        for h in range(H):
            qr[h][rows, :] = (_dot(lhs, pltpu.bitcast(wqp[h], bf16)) * QSCALE).astype(bf16)
            kr[h][rows, :] = _dot(lhs, pltpu.bitcast(wkp[h], bf16)).astype(bf16)
            vr[h][rows, :] = _dot(lhs, pltpu.bitcast(wvp[h], bf16)).astype(bf16)
        return carry

    lax.fori_loop(0, L0 // PB, pre, 0)
    cp_wo.wait()
    cp_mem.wait()

    rowi = lax.broadcasted_iota(i32, (80, 96), 0)
    coli = lax.broadcasted_iota(i32, (80, 96), 1)
    odd = ((rowi >= 32) & (rowi < 64)) | (rowi >= 72)
    rq = jnp.where(rowi < 64, rowi & (SEG - 1), 64)
    cc = coli - jnp.where(odd, 48, 0)
    real = (cc >= 0) & (cc < M + SEG)
    mask = real & ((cc >= SEG) | (cc <= rq))
    fillv = jnp.where(real, MASKED, -jnp.inf).astype(f32)
    z8 = jnp.zeros((8, DH), f32)
    schedule = _step_schedule()

    def step(j, ph, mem):
        s = 4 * j + ph
        xrow = [L0 + G * s + 8 * i for i in range(3)]
        xslot = [pl.multiple_of(lax.rem(r, R), 8) for r in xrow]
        orow = [pl.multiple_of(128 * j + G * ph + 8 * i, 8) for i in range(3)]
        oslot = [pl.multiple_of(lax.rem(r, R), 8) for r in orow]
        seg = pl.ds(pl.multiple_of(lax.rem(SEG * s, R), SEG), SEG)
        fseg = pl.ds(pl.multiple_of(lax.rem(128 * j + (R - SEG), R), SEG), SEG)
        lhs = jnp.concatenate(
            [mem] + [xn_ref[pl.ds(pl.multiple_of(r, 8), 8), :].astype(f32) for r in xrow],
            axis=0).astype(bf16)
        st = {}

        def proj(h, wref, ring, key, scale=None):
            p = _dot(lhs, pltpu.bitcast(wref[h], bf16))
            if scale is not None:
                p = p * scale
            for i in range(3):
                ring[h][pl.ds(xslot[i], 8), :] = p[8 * (i + 1):8 * (i + 2)].astype(bf16)
            if key == "qm":
                st[key, h] = p[0:8]
            else:
                st[key, h] = jnp.concatenate([p[0:8], z8], axis=0).astype(bf16)

        def qkv(h):
            proj(h, wqp, qr, "qm", QSCALE)
            proj(h, wkp, kr, "km")
            proj(h, wvp, vr, "vm")

        def qk(p):
            h0, h1 = 2 * p, 2 * p + 1
            qm = jnp.concatenate([st.pop(("qm", h0)), st.pop(("qm", h1))], axis=0).astype(bf16)
            q_all = jnp.concatenate([qr[h0][seg, :], qr[h1][seg, :], qm], axis=0)
            k_all = jnp.concatenate(
                [kr[h0][seg, :], st.pop(("km", h0)), kr[h1][seg, :], st.pop(("km", h1))], axis=0)
            sc = lax.dot_general(q_all, k_all, (((1,), (1,)), ((), ())), preferred_element_type=f32)
            sc = jnp.where(mask, sc, fillv)
            e = jnp.exp2(sc - jnp.max(sc, axis=1, keepdims=True))
            l = jnp.sum(e, axis=1, keepdims=True)
            r = pl.reciprocal(l, approx=True)
            st["il", p] = r * (2.0 - l * r)
            st["p", p] = e.astype(bf16)

        def pv(p):
            h0, h1 = 2 * p, 2 * p + 1
            v_all = jnp.concatenate(
                [vr[h0][seg, :], st.pop(("vm", h0)), vr[h1][seg, :], st.pop(("vm", h1))], axis=0)
            o = _dot(st.pop(("p", p)), v_all) * st.pop(("il", p))
            for n, h in enumerate((h0, h1)):
                orr[h][seg, :] = o[SEG * n:SEG * (n + 1)].astype(bf16)
                og = [orr[h][pl.ds(oslot[i], 8), :].astype(f32) for i in range(3)]
                st["lo", h] = jnp.concatenate(
                    [o[2 * SEG + 8 * n:2 * SEG + 8 * (n + 1)]] + og, axis=0).astype(bf16)

        def wo(h):
            t = _dot(st.pop(("lo", h)), pltpu.bitcast(wop[h], bf16))
            st["acc"] = st["acc"] + t if "acc" in st else t

        def fill(n):
            h = (H // 4) * ph + n
            t = _dot(orr[h][fseg, :], pltpu.bitcast(wop[h], bf16))
            st["facc"] = st["facc"] + t if "facc" in st else t

        fns = dict(qkv=qkv, qk=qk, pv=pv, wo=wo, fill=fill)
        for op, arg in schedule:
            fns[op](arg)

        acc = st["acc"]
        for i in range(3):
            rr = pl.ds(orow[i], 8)
            out_s[rr, :] = ((xs[rr, :].astype(f32) + acc_ref[rr, :])
                            + acc[8 * (i + 1):8 * (i + 2)]).astype(bf16)
        if ph == 0:
            facc_ref[...] = st["facc"]
        elif ph < 3:
            facc_ref[...] += st["facc"]
        else:
            rd = pl.ds(pl.multiple_of(jnp.maximum(128 * j - SEG, 0), SEG), SEG)
            wr = pl.ds(pl.multiple_of(jnp.where(j > 0, 128 * j - SEG, S), SEG), SEG)
            out_s[wr, :] = ((xs[rd, :].astype(f32) + acc_ref[rd, :])
                            + (facc_ref[...] + st["facc"])).astype(bf16)
        return acc[0:8]

    def group(j, mem):
        @pl.when(j == 1)
        def _():
            cp_out(0, 3 * SEG).start()

        @pl.when(j > 1)
        def _():
            cp_out(pl.multiple_of(128 * (j - 1) - SEG, SEG), 128).start()

        for ph in range(4):
            mem = step(j, ph, mem)
        return mem

    for h in range(H):
        orr[h][R - SEG:R, :] = jnp.zeros((SEG, DH), bf16)
    lax.fori_loop(0, NSEG // 4, group, mem0_s[...].astype(f32))

    cp_out(S - 128 - SEG, 128).start()
    slot = (S - SEG) % R
    lo = jnp.concatenate([orr[h][slot:slot + SEG, :] for h in range(H)], axis=1)
    t = _dot(lo, pltpu.bitcast(wop[...].reshape(H * DH // 2, D), bf16))
    out_s[S - SEG:S, :] = ((xs[S - SEG:S, :].astype(f32) + acc_ref[S - SEG:S, :]) + t).astype(bf16)
    cp_out(S - SEG, SEG).start()
    pltpu.make_async_copy(out_s.at[pl.ds(0, S), :], out_hbm, sem_out).wait()


@jax.jit
def pallas_parallel_sum__memory_aug_recurrent_mem_tr__dense_activation_gelu__prompt_kernel(
    A_x: jax.Array,
    A_mem0: jax.Array,
    A_Wq: jax.Array,
    A_Wk: jax.Array,
    A_Wv: jax.Array,
    A_Wo: jax.Array,
    A_seg_len: jax.Array,
    B_x: jax.Array,
    B_w1: jax.Array,
    B_b1: jax.Array,
    B_w2: jax.Array,
    B_b2: jax.Array,
):
    del A_seg_len, B_x
    assert A_x.shape == (1, S, D) and A_Wq.shape == (D, H, DH) and B_w1.shape == (D, F)
    hbm = pl.BlockSpec(memory_space=pltpu.HBM)
    vmem, dma = pltpu.VMEM, pltpu.SemaphoreType.DMA
    out = pl.pallas_call(
        _kernel,
        out_shape=jax.ShapeDtypeStruct((S, D), bf16),
        in_specs=[hbm] * 10,
        out_specs=hbm,
        scratch_shapes=[
            vmem((H, D // 2, DH), i32), vmem((H, D // 2, DH), i32), vmem((H, D // 2, DH), i32),
            vmem((H, DH // 2, D), i32), vmem((D // 2, F), i32), vmem((F // 2, D), i32),
            vmem((NRAW + 1, 3, RAWD * H // 2, DH), i32),
            vmem((S, D), bf16), vmem((S + LNT, D), bf16), vmem((S, D), f32),
            vmem((BM // 2, FC), i32), vmem((SEG, D), f32), vmem((S + SEG, D), bf16),
            [vmem((R, DH), bf16)] * H, [vmem((R, DH), bf16)] * H,
            [vmem((R, DH), bf16)] * H, [vmem((R, DH), bf16)] * H,
            vmem((M, D), bf16), vmem((F,), bf16), vmem((D,), bf16),
            vmem((NC, 1, FC), f32), vmem((1, D), f32),
            dma((NR,)), dma((XS,)), dma((NC,)), dma((len(W1S) - 1,)), dma((NC,)),
            dma((NRAW,)), dma((4,)), dma(()),
        ],
        compiler_params=pltpu.CompilerParams(
            vmem_limit_bytes=120 * 1024 * 1024,
            disable_bounds_checks=True,
            flags={"XLA_TPU_EVENLY_DISTRIBUTE_CRITICAL_NODES": True},
        ),
        name="fused",
    )(A_x.reshape(S, D), A_mem0.reshape(M, D),
      A_Wq.reshape(D * H, DH), A_Wk.reshape(D * H, DH), A_Wv.reshape(D * H, DH),
      A_Wo, B_w1, B_b1, B_w2, B_b2)
    return out.reshape(1, S, D)
```

```python
import jax
import jax.numpy as jnp
from jax import lax
import jax.experimental.pallas as pl
import jax.experimental.pallas.tpu as pltpu

S, D, H, DH, M, SEG, F = 2048, 1024, 32, 128, 8, 32, 3584
NSEG = S // SEG
G = 24
L0 = 512
R = 576
PB = 128

BM, FC = 512, 896
NR, NC = S // BM, F // FC
NT = FC // 128
LNT = 256
XS = 4
W1S = (0, 1, 3, NT)
RAWD, NRAW = 80, 13
RAW0 = 3

LOG2E = 1.4426950408889634
QSCALE = DH ** -0.5 * LOG2E
MASKED = -1e9 * LOG2E

bf16, f32, i32 = jnp.bfloat16, jnp.float32, jnp.int32


def _gelu(x):
    c = 0.7978845608028654
    return 0.5 * x * (1.0 + jnp.tanh(c * (x + 0.044715 * (x * x * x))))


def _dot(a, b):
    return jnp.dot(a, b, preferred_element_type=f32)


def _step_schedule():
    a, b, c = 1, 3, 6
    ops = []
    for t in range(H // 2):
        ops.append(("qkv", 2 * t))
        if t >= a:
            ops.append(("qk", t - a))
        ops.append(("qkv", 2 * t + 1))
        if t >= b:
            ops.append(("pv", t - b))
        if t >= c:
            ops.append(("wo", t - c))
    left = {"qk": list(range(H // 2 - a, H // 2)),
            "pv": list(range(H // 2 - b, H // 2)),
            "wo": list(range(H // 2 - c, H // 2))}
    for op in ("pv", "pv", "wo", "qk", "wo", "wo", "pv", "wo", "wo", "wo"):
        ops.append((op, left[op].pop(0)))
    ops.append(("fill", 0))
    assert not any(left.values())
    return ops


def _kernel(x_hbm, mem0_hbm, wq_hbm, wk_hbm, wv_hbm, wo_hbm, w1_hbm, b1_hbm, w2_hbm, b2_hbm,
            out_hbm,
            wqp, wkp, wvp, wop, w1p, w2p, stg,
            xs, xn_ref, acc_ref, hs_ref, facc_ref, out_s,
            qr, kr, vr, orr,
            mem0_s, b1_s, b2_s, b1c, b2r,
            sem_x, sem_x0, sem_w1, sem_w1f, sem_w2, sem_raw, sem_misc, sem_out):

    def cp_x(r):
        rows = pl.ds(r * BM, BM)
        return pltpu.make_async_copy(x_hbm.at[rows, :], xs.at[rows, :], sem_x.at[r])

    def cp_x0(p):
        rows = pl.ds(p * (BM // XS), BM // XS)
        return pltpu.make_async_copy(x_hbm.at[rows, :], xs.at[rows, :], sem_x0.at[p])

    def cp_w1(c):
        cols = pl.ds(c * FC, FC)
        return pltpu.make_async_copy(w1_hbm.at[:, cols], w1p.bitcast(bf16).at[:, cols], sem_w1.at[c])

    def cp_w1f(p):
        cols = pl.ds(W1S[p] * 128, (W1S[p + 1] - W1S[p]) * 128)
        return pltpu.make_async_copy(w1_hbm.at[:, cols], w1p.bitcast(bf16).at[:, cols], sem_w1f.at[p])

    def cp_w2(c):
        rows = pl.ds(c * FC, FC)
        return pltpu.make_async_copy(w2_hbm.at[rows, :], w2p.bitcast(bf16).at[rows, :], sem_w2.at[c])

    def raw_d0(k):
        if isinstance(k, int):
            return min(k * RAWD, D - RAWD)
        return pl.multiple_of(jnp.minimum(k * RAWD, D - RAWD), 16)

    def cp_raw(k, m):
        row0 = raw_d0(k) * H
        if not isinstance(k, int):
            row0 = pl.multiple_of(row0, 16 * H)
        return pltpu.make_async_copy((wq_hbm, wk_hbm, wv_hbm)[m].at[pl.ds(row0, RAWD * H), :],
                                     stg.at[k, m].bitcast(bf16), sem_raw.at[k])

    def cp_out(row0, n):
        rows = pl.ds(row0, n)
        return pltpu.make_async_copy(out_s.at[rows, :], out_hbm.at[rows, :], sem_out)

    cp_wo = pltpu.make_async_copy(wo_hbm, wop.bitcast(bf16), sem_misc.at[0])
    cp_mem = pltpu.make_async_copy(mem0_hbm, mem0_s, sem_misc.at[1])
    cp_b1 = pltpu.make_async_copy(b1_hbm, b1_s, sem_misc.at[2])
    cp_b2 = pltpu.make_async_copy(b2_hbm, b2_s, sem_misc.at[3])

    cp_b2.start()
    cp_b1.start()
    cp_mem.start()
    for p in range(XS):
        cp_x0(p).start()
    for p in range(len(W1S) - 1):
        cp_w1f(p).start()
    cp_w2(0).start()
    cp_w1(1).start()
    cp_w2(1).start()
    cp_x(1).start()
    for c in range(2, NC):
        cp_w1(c).start()
        cp_w2(c).start()
    for r in range(2, NR):
        cp_x(r).start()

    def layernorm(row0, n, dst0):
        x = xs[pl.ds(row0, n), :].astype(f32)
        mu = jnp.mean(x, axis=-1, keepdims=True)
        xc = x - mu
        var = jnp.mean(xc * xc, axis=-1, keepdims=True)
        xn_ref[pl.ds(dst0, n), :] = (xc * lax.rsqrt(var + 1e-5)).astype(bf16)

    def deinterleave(krel, parts):
        d0 = raw_d0(jnp.maximum(krel, 0))
        k = jnp.where(krel < 0, NRAW, krel)
        for (m, g, hp) in parts:
            dst = (wqp, wkp, wvp)[m]
            rows = pl.ds(pl.multiple_of(d0 // 2 + g * 8, 8), 8)
            z = stg[k, m, pl.ds(g * 256 + hp, 16, stride=16), :]
            dst[2 * hp, rows, :] = pltpu.bitcast(z.astype(jnp.int16), i32)
            dst[2 * hp + 1, rows, :] = pltpu.bitcast((z >> 16).astype(jnp.int16), i32)

    nslots = NT + D // 128
    all_parts = [(m, g, hp) for m in range(3) for g in range(RAWD // 16) for hp in range(H // 2)]
    slot_parts = [[] for _ in range(nslots)]
    for idx, part in enumerate(all_parts):
        slot_parts[2 + idx * (nslots - 4) // len(all_parts)].append(part)

    for m in range(3):
        stg[NRAW, m] = jnp.zeros((RAWD * H // 2, DH), i32)
    cp_b2.wait()
    b2r[...] = b2_s[...].astype(f32).reshape(1, D)
    cp_b1.wait()
    b1v = b1_s[...].astype(f32).reshape(1, F)
    for c in range(NC):
        b1c[c] = b1v[:, c * FC:(c + 1) * FC]
    for p in range(XS):
        cp_x0(p).wait()
        for j in range(BM // XS // 128):
            layernorm(p * (BM // XS) + j * 128, 128, p * (BM // XS) + j * 128)
    for k in range(NRAW):
        for m in range(3):
            cp_raw(k, m).start()

    def ffn(i, carry, first=False):
        r, c = i // NC, i % NC
        k = i - RAW0
        if not first:
            @pl.when(r == 0)
            def _():
                cp_w1(c).wait()
                cp_w2(c).wait()

            @pl.when((c == NC - BM // LNT) & (r < NR - 1))
            def _():
                cp_x(r + 1).wait()

            @pl.when(k >= 0)
            def _():
                for m in range(3):
                    cp_raw(k, m).wait()

            @pl.when(i == 2)
            def _():
                cp_wo.start()

            lnv = (r + 1 < NR) & (c >= NC - BM // LNT)
            src = pl.multiple_of(
                jnp.where(lnv, (r + 1) * BM + (c - (NC - BM // LNT)) * LNT, r * BM), 16)
            dst = pl.multiple_of(jnp.where(lnv, src, S), 16)

        def side(slot):
            if first:
                return
            deinterleave(k, slot_parts[slot])
            if slot == 3:
                layernorm(src, LNT, dst)

        rows = pl.ds(pl.multiple_of(r * BM, BM), BM)
        xb = xn_ref[rows, :]
        for j in range(NT):
            if first and j in W1S:
                cp_w1f(W1S.index(j)).wait()
            cols = pl.ds(pl.multiple_of(c * FC + j * 128, 128), 128)
            hj = _dot(xb, pltpu.bitcast(w1p[:, cols], bf16)) + b1c[c, :, j * 128:(j + 1) * 128]
            hs_ref[:, j * 128:(j + 1) * 128] = pltpu.bitcast(_gelu(hj).astype(bf16), i32)
            side(j)
        if first:
            cp_w2(0).wait()
        h = pltpu.bitcast(hs_ref[...], bf16)
        for n in range(D // 128):
            ncols = slice(n * 128, (n + 1) * 128)
            w2v = pltpu.bitcast(w2p[pl.ds(pl.multiple_of(c * (FC // 2), 8), FC // 2), ncols], bf16)
            if first:
                base = b2r[:, ncols]
            else:
                base = jnp.where(c == 0, jnp.broadcast_to(b2r[:, ncols], (BM, 128)), acc_ref[rows, ncols])
            acc_ref[rows, ncols] = base + _dot(h, w2v)
            side(NT + n)
        return carry

    ffn(0, 0, first=True)
    lax.fori_loop(1, NR * NC, ffn, 0)

    def pre(j, carry):
        rows = pl.ds(pl.multiple_of(j * PB, PB), PB)
        lhs = xn_ref[rows, :]
        for h in range(H):
            qr[h][rows, :] = (_dot(lhs, pltpu.bitcast(wqp[h], bf16)) * QSCALE).astype(bf16)
            kr[h][rows, :] = _dot(lhs, pltpu.bitcast(wkp[h], bf16)).astype(bf16)
            vr[h][rows, :] = _dot(lhs, pltpu.bitcast(wvp[h], bf16)).astype(bf16)
        return carry

    lax.fori_loop(0, L0 // PB, pre, 0)
    cp_wo.wait()
    cp_mem.wait()

    rowi = lax.broadcasted_iota(i32, (80, 96), 0)
    coli = lax.broadcasted_iota(i32, (80, 96), 1)
    odd = ((rowi >= 32) & (rowi < 64)) | (rowi >= 72)
    rq = jnp.where(rowi < 64, rowi & (SEG - 1), 64)
    cc = coli - jnp.where(odd, 48, 0)
    real = (cc >= 0) & (cc < M + SEG)
    mask = real & ((cc >= SEG) | (cc <= rq))
    fillv = jnp.where(real, MASKED, -jnp.inf).astype(f32)
    z8 = jnp.zeros((8, DH), f32)
    schedule = _step_schedule()

    def step(j, ph, mem):
        s = 4 * j + ph
        xrow = [L0 + G * s + 8 * i for i in range(3)]
        xslot = [pl.multiple_of(lax.rem(r, R), 8) for r in xrow]
        orow = [pl.multiple_of(128 * j + G * ph + 8 * i, 8) for i in range(3)]
        oslot = [pl.multiple_of(lax.rem(r, R), 8) for r in orow]
        seg = pl.ds(pl.multiple_of(lax.rem(SEG * s, R), SEG), SEG)
        fseg = pl.ds(pl.multiple_of(lax.rem(128 * j + (R - SEG), R), SEG), SEG)
        lhs = jnp.concatenate(
            [mem] + [xn_ref[pl.ds(pl.multiple_of(r, 8), 8), :].astype(f32) for r in xrow],
            axis=0).astype(bf16)
        st = {}

        def proj(h, wref, ring, key, scale=None):
            p = _dot(lhs, pltpu.bitcast(wref[h], bf16))
            if scale is not None:
                p = p * scale
            for i in range(3):
                ring[h][pl.ds(xslot[i], 8), :] = p[8 * (i + 1):8 * (i + 2)].astype(bf16)
            if key == "qm":
                st[key, h] = p[0:8]
            else:
                st[key, h] = jnp.concatenate([p[0:8], z8], axis=0).astype(bf16)

        def qkv(h):
            proj(h, wqp, qr, "qm", QSCALE)
            proj(h, wkp, kr, "km")
            proj(h, wvp, vr, "vm")

        def qk(p):
            h0, h1 = 2 * p, 2 * p + 1
            qm = jnp.concatenate([st.pop(("qm", h0)), st.pop(("qm", h1))], axis=0).astype(bf16)
            q_all = jnp.concatenate([qr[h0][seg, :], qr[h1][seg, :], qm], axis=0)
            k_all = jnp.concatenate(
                [kr[h0][seg, :], st.pop(("km", h0)), kr[h1][seg, :], st.pop(("km", h1))], axis=0)
            sc = lax.dot_general(q_all, k_all, (((1,), (1,)), ((), ())), preferred_element_type=f32)
            sc = jnp.where(mask, sc, fillv)
            e = jnp.exp2(sc - jnp.max(sc, axis=1, keepdims=True))
            l = jnp.sum(e, axis=1, keepdims=True)
            r = pl.reciprocal(l, approx=True)
            st["il", p] = r * (2.0 - l * r)
            st["p", p] = e.astype(bf16)

        def pv(p):
            h0, h1 = 2 * p, 2 * p + 1
            v_all = jnp.concatenate(
                [vr[h0][seg, :], st.pop(("vm", h0)), vr[h1][seg, :], st.pop(("vm", h1))], axis=0)
            o = _dot(st.pop(("p", p)), v_all) * st.pop(("il", p))
            for n, h in enumerate((h0, h1)):
                orr[h][seg, :] = o[SEG * n:SEG * (n + 1)].astype(bf16)
                og = [orr[h][pl.ds(oslot[i], 8), :].astype(f32) for i in range(3)]
                st["lo", h] = jnp.concatenate(
                    [o[2 * SEG + 8 * n:2 * SEG + 8 * (n + 1)]] + og, axis=0).astype(bf16)

        def wo(p):
            h0, h1 = 2 * p, 2 * p + 1
            lo = jnp.concatenate([st.pop(("lo", h0)), st.pop(("lo", h1))], axis=1)
            t = _dot(lo, pltpu.bitcast(wop[h0:h0 + 2].reshape(DH, D), bf16))
            st["acc"] = st["acc"] + t if "acc" in st else t

        def fill(_):
            h0 = (H // 4) * ph
            lo = jnp.concatenate([orr[h][fseg, :] for h in range(h0, h0 + H // 4)], axis=1)
            st["facc"] = _dot(lo, pltpu.bitcast(wop[h0:h0 + H // 4].reshape(H // 4 * DH // 2, D), bf16))

        fns = dict(qkv=qkv, qk=qk, pv=pv, wo=wo, fill=fill)
        for op, arg in schedule:
            fns[op](arg)

        acc = st["acc"]
        for i in range(3):
            rr = pl.ds(orow[i], 8)
            out_s[rr, :] = ((xs[rr, :].astype(f32) + acc_ref[rr, :])
                            + acc[8 * (i + 1):8 * (i + 2)]).astype(bf16)
        if ph == 0:
            facc_ref[...] = st["facc"]
        elif ph < 3:
            facc_ref[...] += st["facc"]
        else:
            rd = pl.ds(pl.multiple_of(jnp.maximum(128 * j - SEG, 0), SEG), SEG)
            wr = pl.ds(pl.multiple_of(jnp.where(j > 0, 128 * j - SEG, S), SEG), SEG)
            out_s[wr, :] = ((xs[rd, :].astype(f32) + acc_ref[rd, :])
                            + (facc_ref[...] + st["facc"])).astype(bf16)
        return acc[0:8]

    def group(j, mem):
        @pl.when(j == 1)
        def _():
            cp_out(0, 3 * SEG).start()

        @pl.when(j > 1)
        def _():
            cp_out(pl.multiple_of(128 * (j - 1) - SEG, SEG), 128).start()

        for ph in range(4):
            mem = step(j, ph, mem)
        return mem

    for h in range(H):
        orr[h][R - SEG:R, :] = jnp.zeros((SEG, DH), bf16)
    lax.fori_loop(0, NSEG // 4, group, mem0_s[...].astype(f32))

    cp_out(S - 128 - SEG, 128).start()
    slot = (S - SEG) % R
    lo = jnp.concatenate([orr[h][slot:slot + SEG, :] for h in range(H)], axis=1)
    t = _dot(lo, pltpu.bitcast(wop[...].reshape(H * DH // 2, D), bf16))
    out_s[S - SEG:S, :] = ((xs[S - SEG:S, :].astype(f32) + acc_ref[S - SEG:S, :]) + t).astype(bf16)
    cp_out(S - SEG, SEG).start()
    pltpu.make_async_copy(out_s.at[pl.ds(0, S), :], out_hbm, sem_out).wait()


@jax.jit
def pallas_parallel_sum__memory_aug_recurrent_mem_tr__dense_activation_gelu__prompt_kernel(
    A_x: jax.Array,
    A_mem0: jax.Array,
    A_Wq: jax.Array,
    A_Wk: jax.Array,
    A_Wv: jax.Array,
    A_Wo: jax.Array,
    A_seg_len: jax.Array,
    B_x: jax.Array,
    B_w1: jax.Array,
    B_b1: jax.Array,
    B_w2: jax.Array,
    B_b2: jax.Array,
):
    del A_seg_len, B_x
    assert A_x.shape == (1, S, D) and A_Wq.shape == (D, H, DH) and B_w1.shape == (D, F)
    hbm = pl.BlockSpec(memory_space=pltpu.HBM)
    vmem, dma = pltpu.VMEM, pltpu.SemaphoreType.DMA
    out = pl.pallas_call(
        _kernel,
        out_shape=jax.ShapeDtypeStruct((S, D), bf16),
        in_specs=[hbm] * 10,
        out_specs=hbm,
        scratch_shapes=[
            vmem((H, D // 2, DH), i32), vmem((H, D // 2, DH), i32), vmem((H, D // 2, DH), i32),
            vmem((H, DH // 2, D), i32), vmem((D // 2, F), i32), vmem((F // 2, D), i32),
            vmem((NRAW + 1, 3, RAWD * H // 2, DH), i32),
            vmem((S, D), bf16), vmem((S + LNT, D), bf16), vmem((S, D), f32),
            vmem((BM // 2, FC), i32), vmem((SEG, D), f32), vmem((S + SEG, D), bf16),
            [vmem((R, DH), bf16)] * H, [vmem((R, DH), bf16)] * H,
            [vmem((R, DH), bf16)] * H, [vmem((R, DH), bf16)] * H,
            vmem((M, D), bf16), vmem((F,), bf16), vmem((D,), bf16),
            vmem((NC, 1, FC), f32), vmem((1, D), f32),
            dma((NR,)), dma((XS,)), dma((NC,)), dma((len(W1S) - 1,)), dma((NC,)),
            dma((NRAW,)), dma((4,)), dma(()),
        ],
        compiler_params=pltpu.CompilerParams(
            vmem_limit_bytes=120 * 1024 * 1024,
            disable_bounds_checks=True,
            flags={"XLA_TPU_EVENLY_DISTRIBUTE_CRITICAL_NODES": True},
        ),
        name="fused",
    )(A_x.reshape(S, D), A_mem0.reshape(M, D),
      A_Wq.reshape(D * H, DH), A_Wk.reshape(D * H, DH), A_Wv.reshape(D * H, DH),
      A_Wo, B_w1, B_b1, B_w2, B_b2)
    return out.reshape(1, S, D)
```

```python
import jax
import jax.numpy as jnp
from jax import lax
import jax.experimental.pallas as pl
import jax.experimental.pallas.tpu as pltpu

S, D, H, DH, M, SEG, F = 2048, 1024, 32, 128, 8, 32, 3584
NSEG = S // SEG
G = 24
L0 = 512
R = 576
PB = 128

BM, FC = 512, 896
NR, NC = S // BM, F // FC
NT = FC // 128
LNT = 256
XS = 4
W1S = (0, 1, 3, NT)
RAWD, NRAW = 96, 11

LOG2E = 1.4426950408889634
QSCALE = DH ** -0.5 * LOG2E
MASKED = -1e9 * LOG2E

bf16, f32, i32 = jnp.bfloat16, jnp.float32, jnp.int32


def _gelu(x):
    c = 0.7978845608028654
    return 0.5 * x * (1.0 + jnp.tanh(c * (x + 0.044715 * (x * x * x))))


def _dot(a, b):
    return jnp.dot(a, b, preferred_element_type=f32)


def _step_schedule():
    a, b, c = 1, 3, 6
    ops = []
    for t in range(H // 2):
        ops.append(("qkv", 2 * t))
        if t >= a:
            ops.append(("qk", t - a))
        ops.append(("qkv", 2 * t + 1))
        if t >= b:
            ops.append(("pv", t - b))
        if t >= c:
            ops.append(("wo", t - c))
    left = {"qk": list(range(H // 2 - a, H // 2)),
            "pv": list(range(H // 2 - b, H // 2)),
            "wo": list(range(H // 2 - c, H // 2))}
    for op in ("pv", "pv", "wo", "qk", "wo", "wo", "pv", "wo", "wo", "wo"):
        ops.append((op, left[op].pop(0)))
    ops.append(("fill", 0))
    assert not any(left.values())
    return ops


def _kernel(x_hbm, mem0_hbm, wq_hbm, wk_hbm, wv_hbm, wo_hbm, w1_hbm, b1_hbm, w2_hbm, b2_hbm,
            out_hbm,
            wqp, wkp, wvp, wop, w1p, w2p, stg,
            xs, xn_ref, acc_ref, hs_ref, facc_ref, out_s,
            qr, kr, vr, orr,
            mem0_s, b1_s, b2_s, b1c, b2r,
            sem_x, sem_x0, sem_w1, sem_w1f, sem_w2, sem_raw, sem_misc, sem_out):

    def cp_x(r):
        rows = pl.ds(r * BM, BM)
        return pltpu.make_async_copy(x_hbm.at[rows, :], xs.at[rows, :], sem_x.at[r])

    def cp_x0(p):
        rows = pl.ds(p * (BM // XS), BM // XS)
        return pltpu.make_async_copy(x_hbm.at[rows, :], xs.at[rows, :], sem_x0.at[p])

    def cp_w1(c):
        cols = pl.ds(c * FC, FC)
        return pltpu.make_async_copy(w1_hbm.at[:, cols], w1p.bitcast(bf16).at[:, cols], sem_w1.at[c])

    def cp_w1f(p):
        cols = pl.ds(W1S[p] * 128, (W1S[p + 1] - W1S[p]) * 128)
        return pltpu.make_async_copy(w1_hbm.at[:, cols], w1p.bitcast(bf16).at[:, cols], sem_w1f.at[p])

    def cp_w2(c):
        rows = pl.ds(c * FC, FC)
        return pltpu.make_async_copy(w2_hbm.at[rows, :], w2p.bitcast(bf16).at[rows, :], sem_w2.at[c])

    def raw_d0(k):
        if isinstance(k, int):
            return min(k * RAWD, D - RAWD)
        return pl.multiple_of(jnp.minimum(k * RAWD, D - RAWD), 16)

    def cp_raw(k, m):
        row0 = raw_d0(k) * H
        if not isinstance(k, int):
            row0 = pl.multiple_of(row0, 16 * H)
        return pltpu.make_async_copy((wq_hbm, wk_hbm, wv_hbm)[m].at[pl.ds(row0, RAWD * H), :],
                                     stg.at[k, m].bitcast(bf16), sem_raw.at[k])

    def cp_out(row0, n):
        rows = pl.ds(row0, n)
        return pltpu.make_async_copy(out_s.at[rows, :], out_hbm.at[rows, :], sem_out)

    cp_wo = pltpu.make_async_copy(wo_hbm, wop.bitcast(bf16), sem_misc.at[0])
    cp_mem = pltpu.make_async_copy(mem0_hbm, mem0_s, sem_misc.at[1])
    cp_b1 = pltpu.make_async_copy(b1_hbm, b1_s, sem_misc.at[2])
    cp_b2 = pltpu.make_async_copy(b2_hbm, b2_s, sem_misc.at[3])

    cp_b2.start()
    cp_b1.start()
    cp_mem.start()
    for p in range(XS):
        cp_x0(p).start()
    for p in range(len(W1S) - 1):
        cp_w1f(p).start()
    cp_w2(0).start()
    cp_w1(1).start()
    cp_w2(1).start()
    cp_x(1).start()
    for c in range(2, NC):
        cp_w1(c).start()
        cp_w2(c).start()
    for r in range(2, NR):
        cp_x(r).start()

    def layernorm(row0, n, dst0):
        x = xs[pl.ds(row0, n), :].astype(f32)
        mu = jnp.mean(x, axis=-1, keepdims=True)
        xc = x - mu
        var = jnp.mean(xc * xc, axis=-1, keepdims=True)
        xn_ref[pl.ds(dst0, n), :] = (xc * lax.rsqrt(var + 1e-5)).astype(bf16)

    def deinterleave(krel, parts):
        k = jnp.minimum(krel, NRAW - 1)
        d0 = raw_d0(k)
        for (m, g, hp) in parts:
            dst = (wqp, wkp, wvp)[m]
            rows = pl.ds(pl.multiple_of(d0 // 2 + g * 8, 8), 8)
            z = stg[k, m, pl.ds(g * 256 + hp, 16, stride=16), :]
            dst[2 * hp, rows, :] = pltpu.bitcast(z.astype(jnp.int16), i32)
            dst[2 * hp + 1, rows, :] = pltpu.bitcast((z >> 16).astype(jnp.int16), i32)

    nslots = NT + D // 128
    all_parts = [(m, g, hp) for m in range(3) for g in range(RAWD // 16) for hp in range(H // 2)]
    slot_parts = [[] for _ in range(nslots)]
    for idx, part in enumerate(all_parts):
        slot_parts[3 + idx * (nslots - 6) // len(all_parts)].append(part)

    cp_b2.wait()
    b2r[...] = b2_s[...].astype(f32).reshape(1, D)
    cp_b1.wait()
    b1v = b1_s[...].astype(f32).reshape(1, F)
    for c in range(NC):
        b1c[c] = b1v[:, c * FC:(c + 1) * FC]
    for p in range(XS):
        cp_x0(p).wait()
        for j in range(BM // XS // 128):
            layernorm(p * (BM // XS) + j * 128, 128, p * (BM // XS) + j * 128)
    for k in range(NRAW):
        for m in range(3):
            cp_raw(k, m).start()

    def ffn_block(r, c, first=False, may_be_first_chunk=False, side=None):
        rows = pl.ds(pl.multiple_of(r * BM, BM), BM)
        xb = xn_ref[rows, :]
        for j in range(NT):
            if first and j in W1S:
                cp_w1f(W1S.index(j)).wait()
            cols = pl.ds(pl.multiple_of(c * FC + j * 128, 128), 128)
            hj = _dot(xb, pltpu.bitcast(w1p[:, cols], bf16)) + b1c[c, :, j * 128:(j + 1) * 128]
            hs_ref[:, j * 128:(j + 1) * 128] = pltpu.bitcast(_gelu(hj).astype(bf16), i32)
            if side:
                side(j)
        if first:
            cp_w2(0).wait()
        h = pltpu.bitcast(hs_ref[...], bf16)
        for n in range(D // 128):
            ncols = slice(n * 128, (n + 1) * 128)
            w2v = pltpu.bitcast(w2p[pl.ds(pl.multiple_of(c * (FC // 2), 8), FC // 2), ncols], bf16)
            if first:
                base = b2r[:, ncols]
            elif may_be_first_chunk:
                base = jnp.where(c == 0, jnp.broadcast_to(b2r[:, ncols], (BM, 128)), acc_ref[rows, ncols])
            else:
                base = acc_ref[rows, ncols]
            acc_ref[rows, ncols] = base + _dot(h, w2v)
            if side:
                side(NT + n)

    def ln_rows(valid, row0, r):
        src = pl.multiple_of(jnp.where(valid, row0, r * BM), 16)
        return src, pl.multiple_of(jnp.where(valid, src, S), 16)

    def ffn_a(c, carry):
        cp_w1(c).wait()
        cp_w2(c).wait()

        @pl.when(c == NC - BM // LNT)
        def _():
            cp_x(1).wait()

        src, dst = ln_rows(c >= NC - BM // LNT, BM + (c - (NC - BM // LNT)) * LNT, 0)

        def side(slot):
            if slot == 3:
                layernorm(src, LNT, dst)
        ffn_block(0, c, side=side)
        return carry

    def ffn_b(t, carry):
        r = 1 + t // 2
        u = t % 2
        k0 = 2 * t

        @pl.when((u == 0) & (r < NR - 1))
        def _():
            cp_x(r + 1).wait()

        for e in range(2):
            @pl.when(k0 + e < NRAW)
            def _():
                for m in range(3):
                    cp_raw(k0 + e, m).wait()

        @pl.when(t == 0)
        def _():
            cp_wo.start()

        src, dst = ln_rows(r + 1 < NR, (r + 1) * BM + u * LNT, r)
        for e in range(2):
            def side(slot, e=e):
                deinterleave(k0 + e, slot_parts[slot])
                if slot == 3 and e == 1:
                    layernorm(src, LNT, dst)
            ffn_block(r, 2 * u + e, may_be_first_chunk=(e == 0), side=side)
        return carry

    ffn_block(0, 0, first=True)
    lax.fori_loop(1, NC, ffn_a, 0)
    lax.fori_loop(0, (NR - 1) * NC // 2, ffn_b, 0)

    def pre(j, carry):
        rows = pl.ds(pl.multiple_of(j * PB, PB), PB)
        lhs = xn_ref[rows, :]
        for h in range(H):
            qr[h][rows, :] = (_dot(lhs, pltpu.bitcast(wqp[h], bf16)) * QSCALE).astype(bf16)
            kr[h][rows, :] = _dot(lhs, pltpu.bitcast(wkp[h], bf16)).astype(bf16)
            vr[h][rows, :] = _dot(lhs, pltpu.bitcast(wvp[h], bf16)).astype(bf16)
        return carry

    lax.fori_loop(0, L0 // PB, pre, 0)
    cp_wo.wait()
    cp_mem.wait()

    rowi = lax.broadcasted_iota(i32, (80, 96), 0)
    coli = lax.broadcasted_iota(i32, (80, 96), 1)
    odd = ((rowi >= 32) & (rowi < 64)) | (rowi >= 72)
    rq = jnp.where(rowi < 64, rowi & (SEG - 1), 64)
    cc = coli - jnp.where(odd, 48, 0)
    real = (cc >= 0) & (cc < M + SEG)
    mask = real & ((cc >= SEG) | (cc <= rq))
    fillv = jnp.where(real, MASKED, -jnp.inf).astype(f32)
    z8 = jnp.zeros((8, DH), f32)
    schedule = _step_schedule()

    def step(j, ph, mem):
        s = 4 * j + ph
        xrow = [L0 + G * s + 8 * i for i in range(3)]
        xslot = [pl.multiple_of(lax.rem(r, R), 8) for r in xrow]
        orow = [pl.multiple_of(128 * j + G * ph + 8 * i, 8) for i in range(3)]
        oslot = [pl.multiple_of(lax.rem(r, R), 8) for r in orow]
        seg = pl.ds(pl.multiple_of(lax.rem(SEG * s, R), SEG), SEG)
        fseg = pl.ds(pl.multiple_of(lax.rem(128 * j + (R - SEG), R), SEG), SEG)
        lhs = jnp.concatenate(
            [mem] + [xn_ref[pl.ds(pl.multiple_of(r, 8), 8), :].astype(f32) for r in xrow],
            axis=0).astype(bf16)
        st = {}

        def proj(h, wref, ring, key, scale=None):
            p = _dot(lhs, pltpu.bitcast(wref[h], bf16))
            if scale is not None:
                p = p * scale
            for i in range(3):
                ring[h][pl.ds(xslot[i], 8), :] = p[8 * (i + 1):8 * (i + 2)].astype(bf16)
            if key == "qm":
                st[key, h] = p[0:8]
            else:
                st[key, h] = jnp.concatenate([p[0:8], z8], axis=0).astype(bf16)

        def qkv(h):
            proj(h, wqp, qr, "qm", QSCALE)
            proj(h, wkp, kr, "km")
            proj(h, wvp, vr, "vm")

        def qk(p):
            h0, h1 = 2 * p, 2 * p + 1
            qm = jnp.concatenate([st.pop(("qm", h0)), st.pop(("qm", h1))], axis=0).astype(bf16)
            q_all = jnp.concatenate([qr[h0][seg, :], qr[h1][seg, :], qm], axis=0)
            k_all = jnp.concatenate(
                [kr[h0][seg, :], st.pop(("km", h0)), kr[h1][seg, :], st.pop(("km", h1))], axis=0)
            sc = lax.dot_general(q_all, k_all, (((1,), (1,)), ((), ())), preferred_element_type=f32)
            sc = jnp.where(mask, sc, fillv)
            e = jnp.exp2(sc - jnp.max(sc, axis=1, keepdims=True))
            l = jnp.sum(e, axis=1, keepdims=True)
            r = pl.reciprocal(l, approx=True)
            st["il", p] = r * (2.0 - l * r)
            st["p", p] = e.astype(bf16)

        def pv(p):
            h0, h1 = 2 * p, 2 * p + 1
            v_all = jnp.concatenate(
                [vr[h0][seg, :], st.pop(("vm", h0)), vr[h1][seg, :], st.pop(("vm", h1))], axis=0)
            o = _dot(st.pop(("p", p)), v_all) * st.pop(("il", p))
            for n, h in enumerate((h0, h1)):
                orr[h][seg, :] = o[SEG * n:SEG * (n + 1)].astype(bf16)
                og = [orr[h][pl.ds(oslot[i], 8), :].astype(f32) for i in range(3)]
                st["lo", h] = jnp.concatenate(
                    [o[2 * SEG + 8 * n:2 * SEG + 8 * (n + 1)]] + og, axis=0).astype(bf16)

        def wo(p):
            h0, h1 = 2 * p, 2 * p + 1
            lo = jnp.concatenate([st.pop(("lo", h0)), st.pop(("lo", h1))], axis=1)
            t = _dot(lo, pltpu.bitcast(wop[h0:h0 + 2].reshape(DH, D), bf16))
            st["acc"] = st["acc"] + t if "acc" in st else t

        def fill(_):
            h0 = (H // 4) * ph
            lo = jnp.concatenate([orr[h][fseg, :] for h in range(h0, h0 + H // 4)], axis=1)
            st["facc"] = _dot(lo, pltpu.bitcast(wop[h0:h0 + H // 4].reshape(H // 4 * DH // 2, D), bf16))

        fns = dict(qkv=qkv, qk=qk, pv=pv, wo=wo, fill=fill)
        for op, arg in schedule:
            fns[op](arg)

        acc = st["acc"]
        for i in range(3):
            rr = pl.ds(orow[i], 8)
            out_s[rr, :] = ((xs[rr, :].astype(f32) + acc_ref[rr, :])
                            + acc[8 * (i + 1):8 * (i + 2)]).astype(bf16)
        if ph == 0:
            facc_ref[...] = st["facc"]
        elif ph < 3:
            facc_ref[...] += st["facc"]
        else:
            rd = pl.ds(pl.multiple_of(jnp.maximum(128 * j - SEG, 0), SEG), SEG)
            wr = pl.ds(pl.multiple_of(jnp.where(j > 0, 128 * j - SEG, S), SEG), SEG)
            out_s[wr, :] = ((xs[rd, :].astype(f32) + acc_ref[rd, :])
                            + (facc_ref[...] + st["facc"])).astype(bf16)
        return acc[0:8]

    def group(j, mem):
        @pl.when(j == 1)
        def _():
            cp_out(0, 3 * SEG).start()

        @pl.when(j > 1)
        def _():
            cp_out(pl.multiple_of(128 * (j - 1) - SEG, SEG), 128).start()

        for ph in range(4):
            mem = step(j, ph, mem)
        return mem

    for h in range(H):
        orr[h][R - SEG:R, :] = jnp.zeros((SEG, DH), bf16)
    lax.fori_loop(0, NSEG // 4, group, mem0_s[...].astype(f32))

    cp_out(S - 128 - SEG, 128).start()
    slot = (S - SEG) % R
    lo = jnp.concatenate([orr[h][slot:slot + SEG, :] for h in range(H)], axis=1)
    t = _dot(lo, pltpu.bitcast(wop[...].reshape(H * DH // 2, D), bf16))
    out_s[S - SEG:S, :] = ((xs[S - SEG:S, :].astype(f32) + acc_ref[S - SEG:S, :]) + t).astype(bf16)
    cp_out(S - SEG, SEG).start()
    pltpu.make_async_copy(out_s.at[pl.ds(0, S), :], out_hbm, sem_out).wait()


@jax.jit
def pallas_parallel_sum__memory_aug_recurrent_mem_tr__dense_activation_gelu__prompt_kernel(
    A_x: jax.Array,
    A_mem0: jax.Array,
    A_Wq: jax.Array,
    A_Wk: jax.Array,
    A_Wv: jax.Array,
    A_Wo: jax.Array,
    A_seg_len: jax.Array,
    B_x: jax.Array,
    B_w1: jax.Array,
    B_b1: jax.Array,
    B_w2: jax.Array,
    B_b2: jax.Array,
):
    del A_seg_len, B_x
    assert A_x.shape == (1, S, D) and A_Wq.shape == (D, H, DH) and B_w1.shape == (D, F)
    hbm = pl.BlockSpec(memory_space=pltpu.HBM)
    vmem, dma = pltpu.VMEM, pltpu.SemaphoreType.DMA
    out = pl.pallas_call(
        _kernel,
        out_shape=jax.ShapeDtypeStruct((S, D), bf16),
        in_specs=[hbm] * 10,
        out_specs=hbm,
        scratch_shapes=[
            vmem((H, D // 2, DH), i32), vmem((H, D // 2, DH), i32), vmem((H, D // 2, DH), i32),
            vmem((H, DH // 2, D), i32), vmem((D // 2, F), i32), vmem((F // 2, D), i32),
            vmem((NRAW, 3, RAWD * H // 2, DH), i32),
            vmem((S, D), bf16), vmem((S + LNT, D), bf16), vmem((S, D), f32),
            vmem((BM // 2, FC), i32), vmem((SEG, D), f32), vmem((S + SEG, D), bf16),
            [vmem((R, DH), bf16)] * H, [vmem((R, DH), bf16)] * H,
            [vmem((R, DH), bf16)] * H, [vmem((R, DH), bf16)] * H,
            vmem((M, D), bf16), vmem((F,), bf16), vmem((D,), bf16),
            vmem((NC, 1, FC), f32), vmem((1, D), f32),
            dma((NR,)), dma((XS,)), dma((NC,)), dma((len(W1S) - 1,)), dma((NC,)),
            dma((NRAW,)), dma((4,)), dma(()),
        ],
        compiler_params=pltpu.CompilerParams(
            vmem_limit_bytes=120 * 1024 * 1024,
            disable_bounds_checks=True,
            flags={"XLA_TPU_EVENLY_DISTRIBUTE_CRITICAL_NODES": True},
        ),
        name="fused",
    )(A_x.reshape(S, D), A_mem0.reshape(M, D),
      A_Wq.reshape(D * H, DH), A_Wk.reshape(D * H, DH), A_Wv.reshape(D * H, DH),
      A_Wo, B_w1, B_b1, B_w2, B_b2)
    return out.reshape(1, S, D)
```

```python
import jax
import jax.numpy as jnp
from jax import lax
import jax.experimental.pallas as pl
import jax.experimental.pallas.tpu as pltpu

S, D, H, DH, M, SEG, F = 2048, 1024, 32, 128, 8, 32, 3584
NSEG = S // SEG
G = 24
L0 = 512
R = 576
PB = 64

BM, FC = 512, 896
NR, NC = S // BM, F // FC
NT = FC // 128
LNT = 256
XS = 4
W1S = (0, 1, 3, NT)
RAWD, NRAW = 96, 11

LOG2E = 1.4426950408889634
QSCALE = DH ** -0.5 * LOG2E
MASKED = -1e9 * LOG2E

bf16, f32, i32 = jnp.bfloat16, jnp.float32, jnp.int32


def _gelu(x):
    c = 0.7978845608028654
    return 0.5 * x * (1.0 + jnp.tanh(c * (x + 0.044715 * (x * x * x))))


def _dot(a, b):
    return jnp.dot(a, b, preferred_element_type=f32)


def _step_schedule(filler=True):
    a, b, c = 1, 3, 6
    ops = []
    for t in range(H // 2):
        ops.append(("qkv", 2 * t))
        if t >= a:
            ops.append(("qk", t - a))
        ops.append(("qkv", 2 * t + 1))
        if t >= b:
            ops.append(("pv", t - b))
        if t >= c:
            ops.append(("wo", t - c))
    left = {"qk": list(range(H // 2 - a, H // 2)),
            "pv": list(range(H // 2 - b, H // 2)),
            "wo": list(range(H // 2 - c, H // 2))}
    for op in ("pv", "pv", "wo", "qk", "wo", "wo", "pv", "wo", "wo", "wo"):
        ops.append((op, left[op].pop(0)))
    if filler:
        ops.append(("fill", 0))
    assert not any(left.values())
    return ops


def _kernel(x_hbm, mem0_hbm, wq_hbm, wk_hbm, wv_hbm, wo_hbm, w1_hbm, b1_hbm, w2_hbm, b2_hbm,
            out_hbm,
            wqp, wkp, wvp, wop, w1p, w2p, stg,
            xs, xn_ref, acc_ref, hs_ref, facc_ref, out_s,
            qr, kr, vr, orr,
            mem0_s, b1_s, b2_s, b1c, b2r,
            sem_x, sem_x0, sem_w1, sem_w1f, sem_w2, sem_raw, sem_misc, sem_out):

    def cp_x(r):
        rows = pl.ds(r * BM, BM)
        return pltpu.make_async_copy(x_hbm.at[rows, :], xs.at[rows, :], sem_x.at[r])

    def cp_x0(p):
        rows = pl.ds(p * (BM // XS), BM // XS)
        return pltpu.make_async_copy(x_hbm.at[rows, :], xs.at[rows, :], sem_x0.at[p])

    def cp_w1(c):
        cols = pl.ds(c * FC, FC)
        return pltpu.make_async_copy(w1_hbm.at[:, cols], w1p.bitcast(bf16).at[:, cols], sem_w1.at[c])

    def cp_w1f(p):
        cols = pl.ds(W1S[p] * 128, (W1S[p + 1] - W1S[p]) * 128)
        return pltpu.make_async_copy(w1_hbm.at[:, cols], w1p.bitcast(bf16).at[:, cols], sem_w1f.at[p])

    def cp_w2(c):
        rows = pl.ds(c * FC, FC)
        return pltpu.make_async_copy(w2_hbm.at[rows, :], w2p.bitcast(bf16).at[rows, :], sem_w2.at[c])

    def raw_d0(k):
        if isinstance(k, int):
            return min(k * RAWD, D - RAWD)
        return pl.multiple_of(jnp.minimum(k * RAWD, D - RAWD), 16)

    def cp_raw(k, m):
        row0 = raw_d0(k) * H
        if not isinstance(k, int):
            row0 = pl.multiple_of(row0, 16 * H)
        return pltpu.make_async_copy((wq_hbm, wk_hbm, wv_hbm)[m].at[pl.ds(row0, RAWD * H), :],
                                     stg.at[k, m].bitcast(bf16), sem_raw.at[k])

    def cp_out(row0, n):
        rows = pl.ds(row0, n)
        return pltpu.make_async_copy(out_s.at[rows, :], out_hbm.at[rows, :], sem_out)

    cp_wo = pltpu.make_async_copy(wo_hbm, wop.bitcast(bf16), sem_misc.at[0])
    cp_mem = pltpu.make_async_copy(mem0_hbm, mem0_s, sem_misc.at[1])
    cp_b1 = pltpu.make_async_copy(b1_hbm, b1_s, sem_misc.at[2])
    cp_b2 = pltpu.make_async_copy(b2_hbm, b2_s, sem_misc.at[3])

    cp_b2.start()
    cp_b1.start()
    cp_mem.start()
    for p in range(XS):
        cp_x0(p).start()
    for p in range(len(W1S) - 1):
        cp_w1f(p).start()
    cp_w2(0).start()
    cp_w1(1).start()
    cp_w2(1).start()
    cp_x(1).start()
    for c in range(2, NC):
        cp_w1(c).start()
        cp_w2(c).start()
    for r in range(2, NR):
        cp_x(r).start()

    def layernorm(row0, n, dst0):
        x = xs[pl.ds(row0, n), :].astype(f32)
        mu = jnp.mean(x, axis=-1, keepdims=True)
        xc = x - mu
        var = jnp.mean(xc * xc, axis=-1, keepdims=True)
        xn_ref[pl.ds(dst0, n), :] = (xc * lax.rsqrt(var + 1e-5)).astype(bf16)

    def deinterleave(krel, parts):
        k = jnp.minimum(krel, NRAW - 1)
        d0 = raw_d0(k)
        for (m, g, hp) in parts:
            dst = (wqp, wkp, wvp)[m]
            rows = pl.ds(pl.multiple_of(d0 // 2 + g * 8, 8), 8)
            z = stg[k, m, pl.ds(g * 256 + hp, 16, stride=16), :]
            dst[2 * hp, rows, :] = pltpu.bitcast(z.astype(jnp.int16), i32)
            dst[2 * hp + 1, rows, :] = pltpu.bitcast((z >> 16).astype(jnp.int16), i32)

    nslots = NT + D // 128
    all_parts = [(m, g, hp) for m in range(3) for g in range(RAWD // 16) for hp in range(H // 2)]
    slot_parts = [[] for _ in range(nslots)]
    for idx, part in enumerate(all_parts):
        slot_parts[3 + idx * (nslots - 6) // len(all_parts)].append(part)

    cp_b2.wait()
    b2r[...] = b2_s[...].astype(f32).reshape(1, D)
    cp_b1.wait()
    b1v = b1_s[...].astype(f32).reshape(1, F)
    for c in range(NC):
        b1c[c] = b1v[:, c * FC:(c + 1) * FC]
    for p in range(XS):
        cp_x0(p).wait()
        for j in range(BM // XS // 128):
            layernorm(p * (BM // XS) + j * 128, 128, p * (BM // XS) + j * 128)
    for k in range(NRAW):
        for m in range(3):
            cp_raw(k, m).start()

    def ffn_block(r, c, first=False, may_be_first_chunk=False, side=None):
        rows = pl.ds(pl.multiple_of(r * BM, BM), BM)
        xb = xn_ref[rows, :]
        for j in range(NT):
            if first and j in W1S:
                cp_w1f(W1S.index(j)).wait()
            cols = pl.ds(pl.multiple_of(c * FC + j * 128, 128), 128)
            hj = _dot(xb, pltpu.bitcast(w1p[:, cols], bf16)) + b1c[c, :, j * 128:(j + 1) * 128]
            hs_ref[:, j * 128:(j + 1) * 128] = pltpu.bitcast(_gelu(hj).astype(bf16), i32)
            if side:
                side(j)
        if first:
            cp_w2(0).wait()
        h = pltpu.bitcast(hs_ref[...], bf16)
        for n in range(D // 128):
            ncols = slice(n * 128, (n + 1) * 128)
            w2v = pltpu.bitcast(w2p[pl.ds(pl.multiple_of(c * (FC // 2), 8), FC // 2), ncols], bf16)
            if first:
                base = b2r[:, ncols]
            elif may_be_first_chunk:
                base = jnp.where(c == 0, jnp.broadcast_to(b2r[:, ncols], (BM, 128)), acc_ref[rows, ncols])
            else:
                base = acc_ref[rows, ncols]
            acc_ref[rows, ncols] = base + _dot(h, w2v)
            if side:
                side(NT + n)

    def ln_rows(valid, row0, r):
        src = pl.multiple_of(jnp.where(valid, row0, r * BM), 16)
        return src, pl.multiple_of(jnp.where(valid, src, S), 16)

    def ffn_a(c, carry):
        cp_w1(c).wait()
        cp_w2(c).wait()

        @pl.when(c == NC - BM // LNT)
        def _():
            cp_x(1).wait()

        src, dst = ln_rows(c >= NC - BM // LNT, BM + (c - (NC - BM // LNT)) * LNT, 0)

        def side(slot):
            if slot == 3:
                layernorm(src, LNT, dst)
        ffn_block(0, c, side=side)
        return carry

    def ffn_b(t, carry):
        r = 1 + t // 2
        u = t % 2
        k0 = 2 * t

        @pl.when((u == 0) & (r < NR - 1))
        def _():
            cp_x(r + 1).wait()

        for e in range(2):
            @pl.when(k0 + e < NRAW)
            def _():
                for m in range(3):
                    cp_raw(k0 + e, m).wait()

        @pl.when(t == 0)
        def _():
            cp_wo.start()

        src, dst = ln_rows(r + 1 < NR, (r + 1) * BM + u * LNT, r)
        for e in range(2):
            def side(slot, e=e):
                deinterleave(k0 + e, slot_parts[slot])
                if slot == 3 and e == 1:
                    layernorm(src, LNT, dst)
            ffn_block(r, 2 * u + e, may_be_first_chunk=(e == 0), side=side)
        return carry

    ffn_block(0, 0, first=True)
    lax.fori_loop(1, NC, ffn_a, 0)
    lax.fori_loop(0, (NR - 1) * NC // 2, ffn_b, 0)

    def pre(j, carry):
        rows = pl.ds(pl.multiple_of(j * PB, PB), PB)
        lhs = xn_ref[rows, :]
        for h in range(H):
            qr[h][rows, :] = (_dot(lhs, pltpu.bitcast(wqp[h], bf16)) * QSCALE).astype(bf16)
            kr[h][rows, :] = _dot(lhs, pltpu.bitcast(wkp[h], bf16)).astype(bf16)
            vr[h][rows, :] = _dot(lhs, pltpu.bitcast(wvp[h], bf16)).astype(bf16)
        return carry

    lax.fori_loop(0, L0 // PB, pre, 0)
    cp_wo.wait()
    cp_mem.wait()

    rowi = lax.broadcasted_iota(i32, (80, 96), 0)
    coli = lax.broadcasted_iota(i32, (80, 96), 1)
    odd = ((rowi >= 32) & (rowi < 64)) | (rowi >= 72)
    rq = jnp.where(rowi < 64, rowi & (SEG - 1), 64)
    cc = coli - jnp.where(odd, 48, 0)
    real = (cc >= 0) & (cc < M + SEG)
    mask = real & ((cc >= SEG) | (cc <= rq))
    fillv = jnp.where(real, MASKED, -jnp.inf).astype(f32)
    z8 = jnp.zeros((8, DH), f32)

    def step(j, ph, mem, filler=True):
        s = 4 * j + ph
        xrow = [L0 + G * s + 8 * i for i in range(3)]
        xslot = [pl.multiple_of(lax.rem(r, R), 8) for r in xrow]
        orow = [pl.multiple_of(128 * j + G * ph + 8 * i, 8) for i in range(3)]
        oslot = [pl.multiple_of(lax.rem(r, R), 8) for r in orow]
        seg = pl.ds(pl.multiple_of(lax.rem(SEG * s, R), SEG), SEG)
        if filler:
            fseg = pl.ds(pl.multiple_of(lax.rem(128 * j - SEG, R), SEG), SEG)
        lhs = jnp.concatenate(
            [mem] + [xn_ref[pl.ds(pl.multiple_of(r, 8), 8), :].astype(f32) for r in xrow],
            axis=0).astype(bf16)
        st = {}

        def proj(h, wref, ring, key, scale=None):
            p = _dot(lhs, pltpu.bitcast(wref[h], bf16))
            if scale is not None:
                p = p * scale
            for i in range(3):
                ring[h][pl.ds(xslot[i], 8), :] = p[8 * (i + 1):8 * (i + 2)].astype(bf16)
            if key == "qm":
                st[key, h] = p[0:8]
            else:
                st[key, h] = jnp.concatenate([p[0:8], z8], axis=0).astype(bf16)

        def qkv(h):
            proj(h, wqp, qr, "qm", QSCALE)
            proj(h, wkp, kr, "km")
            proj(h, wvp, vr, "vm")

        def qk(p):
            h0, h1 = 2 * p, 2 * p + 1
            qm = jnp.concatenate([st.pop(("qm", h0)), st.pop(("qm", h1))], axis=0).astype(bf16)
            q_all = jnp.concatenate([qr[h0][seg, :], qr[h1][seg, :], qm], axis=0)
            k_all = jnp.concatenate(
                [kr[h0][seg, :], st.pop(("km", h0)), kr[h1][seg, :], st.pop(("km", h1))], axis=0)
            sc = lax.dot_general(q_all, k_all, (((1,), (1,)), ((), ())), preferred_element_type=f32)
            sc = jnp.where(mask, sc, fillv)
            e = jnp.exp2(sc - jnp.max(sc, axis=1, keepdims=True))
            l = jnp.sum(e, axis=1, keepdims=True)
            r = pl.reciprocal(l, approx=True)
            st["il", p] = r * (2.0 - l * r)
            st["p", p] = e.astype(bf16)

        def pv(p):
            h0, h1 = 2 * p, 2 * p + 1
            v_all = jnp.concatenate(
                [vr[h0][seg, :], st.pop(("vm", h0)), vr[h1][seg, :], st.pop(("vm", h1))], axis=0)
            o = _dot(st.pop(("p", p)), v_all) * st.pop(("il", p))
            for n, h in enumerate((h0, h1)):
                orr[h][seg, :] = o[SEG * n:SEG * (n + 1)].astype(bf16)
                og = [orr[h][pl.ds(oslot[i], 8), :].astype(f32) for i in range(3)]
                st["lo", h] = jnp.concatenate(
                    [o[2 * SEG + 8 * n:2 * SEG + 8 * (n + 1)]] + og, axis=0).astype(bf16)

        def wo(p):
            h0, h1 = 2 * p, 2 * p + 1
            lo = jnp.concatenate([st.pop(("lo", h0)), st.pop(("lo", h1))], axis=1)
            t = _dot(lo, pltpu.bitcast(wop[h0:h0 + 2].reshape(DH, D), bf16))
            st["acc"] = st["acc"] + t if "acc" in st else t

        def fill(_):
            h0 = (H // 4) * ph
            lo = jnp.concatenate([orr[h][fseg, :] for h in range(h0, h0 + H // 4)], axis=1)
            st["facc"] = _dot(lo, pltpu.bitcast(wop[h0:h0 + H // 4].reshape(H // 4 * DH // 2, D), bf16))

        fns = dict(qkv=qkv, qk=qk, pv=pv, wo=wo, fill=fill)
        for op, arg in _step_schedule(filler):
            fns[op](arg)

        acc = st["acc"]
        for i in range(3):
            rr = pl.ds(orow[i], 8)
            out_s[rr, :] = ((xs[rr, :].astype(f32) + acc_ref[rr, :])
                            + acc[8 * (i + 1):8 * (i + 2)]).astype(bf16)
        if filler:
            if ph == 0:
                facc_ref[...] = st["facc"]
            elif ph < 3:
                facc_ref[...] += st["facc"]
            else:
                fr = pl.ds(pl.multiple_of(128 * j - SEG, SEG), SEG)
                out_s[fr, :] = ((xs[fr, :].astype(f32) + acc_ref[fr, :])
                                + (facc_ref[...] + st["facc"])).astype(bf16)
        return acc[0:8]

    def group(j, mem):
        @pl.when(j > 1)
        def _():
            cp_out(pl.multiple_of(128 * (j - 1) - SEG, SEG), 128).start()

        for ph in range(4):
            mem = step(j, ph, mem)
        return mem

    mem = lax.fori_loop(0, 4, lambda ph, mem: step(0, ph, mem, filler=False), mem0_s[...].astype(f32))
    cp_out(0, 3 * SEG).start()
    lax.fori_loop(1, NSEG // 4, group, mem)

    cp_out(S - 128 - SEG, 128).start()
    slot = (S - SEG) % R
    lo = jnp.concatenate([orr[h][slot:slot + SEG, :] for h in range(H)], axis=1)
    t = _dot(lo, pltpu.bitcast(wop[...].reshape(H * DH // 2, D), bf16))
    out_s[S - SEG:S, :] = ((xs[S - SEG:S, :].astype(f32) + acc_ref[S - SEG:S, :]) + t).astype(bf16)
    cp_out(S - SEG, SEG).start()
    pltpu.make_async_copy(out_s.at[pl.ds(0, S), :], out_hbm, sem_out).wait()


@jax.jit
def pallas_parallel_sum__memory_aug_recurrent_mem_tr__dense_activation_gelu__prompt_kernel(
    A_x: jax.Array,
    A_mem0: jax.Array,
    A_Wq: jax.Array,
    A_Wk: jax.Array,
    A_Wv: jax.Array,
    A_Wo: jax.Array,
    A_seg_len: jax.Array,
    B_x: jax.Array,
    B_w1: jax.Array,
    B_b1: jax.Array,
    B_w2: jax.Array,
    B_b2: jax.Array,
):
    del A_seg_len, B_x
    assert A_x.shape == (1, S, D) and A_Wq.shape == (D, H, DH) and B_w1.shape == (D, F)
    hbm = pl.BlockSpec(memory_space=pltpu.HBM)
    vmem, dma = pltpu.VMEM, pltpu.SemaphoreType.DMA
    out = pl.pallas_call(
        _kernel,
        out_shape=jax.ShapeDtypeStruct((S, D), bf16),
        in_specs=[hbm] * 10,
        out_specs=hbm,
        scratch_shapes=[
            vmem((H, D // 2, DH), i32), vmem((H, D // 2, DH), i32), vmem((H, D // 2, DH), i32),
            vmem((H, DH // 2, D), i32), vmem((D // 2, F), i32), vmem((F // 2, D), i32),
            vmem((NRAW, 3, RAWD * H // 2, DH), i32),
            vmem((S, D), bf16), vmem((S + LNT, D), bf16), vmem((S, D), f32),
            vmem((BM // 2, FC), i32), vmem((SEG, D), f32), vmem((S, D), bf16),
            [vmem((R, DH), bf16)] * H, [vmem((R, DH), bf16)] * H,
            [vmem((R, DH), bf16)] * H, [vmem((R, DH), bf16)] * H,
            vmem((M, D), bf16), vmem((F,), bf16), vmem((D,), bf16),
            vmem((NC, 1, FC), f32), vmem((1, D), f32),
            dma((NR,)), dma((XS,)), dma((NC,)), dma((len(W1S) - 1,)), dma((NC,)),
            dma((NRAW,)), dma((4,)), dma(()),
        ],
        compiler_params=pltpu.CompilerParams(
            vmem_limit_bytes=120 * 1024 * 1024,
            disable_bounds_checks=True,
            flags={"XLA_TPU_EVENLY_DISTRIBUTE_CRITICAL_NODES": True},
        ),
        name="fused",
    )(A_x.reshape(S, D), A_mem0.reshape(M, D),
      A_Wq.reshape(D * H, DH), A_Wk.reshape(D * H, DH), A_Wv.reshape(D * H, DH),
      A_Wo, B_w1, B_b1, B_w2, B_b2)
    return out.reshape(1, S, D)
```
